```python
import jax
import jax.numpy as jnp

def _softmax(x, axis=-1):
    return jax.nn.softmax(x, axis=axis)

def _gelu(x):
    return jax.nn.gelu(x, approximate=True)

def _silu(x):
    return jax.nn.silu(x)

def _sigmoid(x):
    return jax.nn.sigmoid(x)

def _layernorm(x, axis=-1, eps=1e-05):
    m = jnp.mean(x, axis=axis, keepdims=True)
    v = jnp.var(x, axis=axis, keepdims=True)
    return (x - m) / jnp.sqrt(v + eps)

def _scatter_add(tgt, idx, src, axis=0):
    return tgt.at[idx].add(src)

def _segment_sum(src, seg, n):
    return jax.ops.segment_sum(src, seg, n)

class _Rng:

    def __init__(self, key):
        self._k = key

    def _next(self):
        self._k, sub = jax.random.split(self._k)
        return sub

    def normal(self, shape):
        return jax.random.normal(self._next(), shape, dtype=jnp.bfloat16)

    def randint(self, lo, hi, shape):
        return jax.random.randint(self._next(), shape, lo, hi, dtype=jnp.int32)

    def uniform(self, shape, lo=0.0, hi=1.0):
        return jax.random.uniform(self._next(), shape, jnp.bfloat16, lo, hi)

    def permutation(self, n):
        return jax.random.permutation(self._next(), n)
kernel_name = 'adaLN_cond__sliding_block_cached__dense_activation_mish__decode'

def setup_inputs():
    _rng = _Rng(jax.random.key(int.from_bytes(__import__("os").urandom(4), "little")))
    _w = lambda a: (lambda t: t.astype(jnp.bfloat16) if jnp.issubdtype(t.dtype, jnp.floating) else t)(jnp.asarray(a))

    def _A_setup():
        B, Sq, D = (1, 1, 640)
        Hq, Hkv, Sk, Dh = (32, 32, 32768, 192)
        assert Hq % Hkv == 0, (Hq, Hkv)
        return {'x': _w((lambda *s: _rng.normal(s) * 0.05)(B, Sq, D)), 'k_cache': _w((lambda *s: _rng.normal(s) * 0.05)(B, Hkv, Sk, Dh)), 'v_cache': _w((lambda *s: _rng.normal(s) * 0.05)(B, Hkv, Sk, Dh)), 'wq': _w((lambda *s: _rng.normal(s) * 0.05)(D, Hq * Dh) * D ** (-0.5)), 'wo': _w((lambda *s: _rng.normal(s) * 0.05)(Hq * Dh, D) * (Hq * Dh) ** (-0.5))}
    _A_in = _A_setup()

    def _B_setup():
        B, S, D, F = (1, 1, 640, 1536)
        return {'x': _w((lambda *s: _rng.normal(s) * 0.05)(B, S, D)), 'w1': _w((lambda *s: _rng.normal(s) * 0.05)(D, F) * D ** (-0.5)), 'b1': _w((lambda *s: _rng.normal(s) * 0.05)(F)), 'w2': _w((lambda *s: _rng.normal(s) * 0.05)(F, D) * F ** (-0.5))}
    _B_in = _B_setup()
    return {'A_x': _A_in['x'], 'A_k_cache': _A_in['k_cache'], 'A_v_cache': _A_in['v_cache'], 'A_wq': _A_in['wq'], 'A_wo': _A_in['wo'], 'B_x': _B_in['x'], 'B_w1': _B_in['w1'], 'B_b1': _B_in['b1'], 'B_w2': _B_in['w2'], 'c': _w((lambda *s: _rng.normal(s) * 0.05)(1, 640)), 'w_mod': _w((lambda *s: _rng.normal(s) * 0.05)(640, 6 * 640) * 640 ** (-0.5))}

def reference(A_x, A_k_cache, A_v_cache, A_wq, A_wo, B_x, B_w1, B_b1, B_w2, c, w_mod):

    def _A_ref(x, k_cache, v_cache, wq, wo):
        B, Sq, D = x.shape
        Hq, Dh = (32, 192)
        Hkv, Sk = (k_cache.shape[1], k_cache.shape[2])
        W = min(4096, max(256, Sk // 4))
        rep = Hq // Hkv
        q = (lambda x, *d: x.transpose(*d))((x @ wq).reshape(B, Sq, Hq, Dh), 0, 2, 1, 3)
        k = jnp.repeat(k_cache[:, :, Sk - W:, :], rep, axis=1)
        v = jnp.repeat(v_cache[:, :, Sk - W:, :], rep, axis=1)
        scores = jnp.einsum('bhqd,bhkd->bhqk', q, k) * Dh ** (-0.5)
        p = _softmax(scores, axis=-1)
        o = jnp.einsum('bhqk,bhkd->bhqd', p, v)
        return (lambda x, *d: x.transpose(*d))(o, 0, 2, 1, 3).reshape(B, Sq, Hq * Dh) @ wo

    def _B_ref(x, w1, b1, w2):
        h = jnp.einsum('bsd,df->bsf', x, w1) + b1
        sp = jnp.log1p(jnp.exp(-jnp.abs(h))) + jnp.where(h > 0, h, jnp.zeros_like(h))
        act = h * jnp.tanh(sp)
        return jnp.einsum('bsf,fd->bsd', act, w2)
    x = A_x
    mod = (_silu(c) @ w_mod).reshape(c.shape[0], 6, 1, -1)
    sa, ca, ga, sb, cb, gb = (mod[:, 0].copy(), mod[:, 1].copy(), mod[:, 2].copy(), mod[:, 3].copy(), mod[:, 4].copy(), mod[:, 5].copy())
    h = _layernorm(x, axis=-1) * (1 + ca) + sa
    x = x + ga * _A_ref(h, A_k_cache, A_v_cache, A_wq, A_wo)
    h = _layernorm(x, axis=-1) * (1 + cb) + sb
    x = x + gb * _B_ref(h, B_w1, B_b1, B_w2)
    return x
```

```python
import functools

import jax
import jax.numpy as jnp
from jax import lax
from jax.experimental import pallas as pl
from jax.experimental.pallas import tpu as pltpu

D = 640
HQ = 32
DH = 192
F = 1536
HD = HQ * DH
GH = 8
GR = GH * DH
UR = 128
UPG = GR // UR
NG = HQ // GH
EPS = 1e-5


def _stride_order(n, step):
    return [(j * step) % n for j in range(n)]


def make(L=3, R=8, kv_order="row", compute=True, dma=True, nochecks=True, b1_mode="2d",
         wq_order=("cls",), wm_order=17, wo_order=13, w1_order=11, w2_order=13, w2_tail=None):
    def kernel(x_hbm, kt_hbm, vt_hbm, wq_hbm, wo_hbm, w1_hbm, b1_hbm, w2_hbm, c_hbm, wm_hbm, o_ref,
               x_v, c_v, b1_v, wma_v, wmb_v, wq_v, wo_v, w1_v, w2_v, ring, mod_s, qbd_s, s_s, p_s, acc_s,
               wsem, rsem):
        sk = kt_hbm.shape[1]
        w = ring.shape[2]
        c0 = sk - w
        half = w // 2

        ctr = [0]

        def start(src, dst, sem):
            if dma:
                pltpu.make_async_copy(src, dst, sem).start(priority=ctr[0] % 2)
            ctr[0] += 1

        def wait(dst, sem):
            if dma:
                pltpu.make_async_copy(dst, dst, sem).wait()

        def issue_unit(src, unit, slot):
            base = pl.multiple_of(unit * UR, UR)
            if kv_order == "row":
                idx = [(r, c) for r in range(UR // 8) for c in range(2)]
            else:
                idx = [(r, c) for c in range(2) for r in range(UR // 8)]
            for r, c in idx:
                start(src.at[pl.ds(base + 8 * r, 8), pl.ds(c0 + c * half, half)],
                      ring.at[slot, pl.ds(8 * r, 8), pl.ds(c * half, half)], rsem.at[slot])

        def pieces_rows(src, dst, sem, rows, step, col0=0):
            n = dst.shape[0] // rows
            ncol = dst.shape[1]
            return [(src.at[pl.ds(j * rows, rows), pl.ds(col0, ncol)], dst.at[pl.ds(j * rows, rows), :], sem)
                    for j in _stride_order(n, step)]

        def issue(pieces):
            for p in pieces:
                start(*p)

        wma_p = pieces_rows(wm_hbm, wma_v, wsem.at[3], 8, wm_order, 0)
        wmb_p = pieces_rows(wm_hbm, wmb_v, wsem.at[4], 8, wm_order, 2 * D)
        if wq_order[0] == "cls":
            order = [k + 16 * j for k2 in range(0, 16, 2) for j in range(15) for k in (k2, k2 + 1)]
        else:
            order = _stride_order(240, wq_order[1])
        wq_p = [(wq_hbm.at[pl.ds((n // 3) * 8, 8), pl.ds((n % 3) * 2048, 2048)],
                 wq_v.at[pl.ds((n // 3) * 8, 8), pl.ds((n % 3) * 2048, 2048)], wsem.at[5]) for n in order]
        wo_p = pieces_rows(wo_hbm, wo_v, wsem.at[6], 32, wo_order)
        w1_p = pieces_rows(w1_hbm, w1_v, wsem.at[7], 16, w1_order)
        w2_p = pieces_rows(w2_hbm, w2_v, wsem.at[8], 32, w2_order)

        start(c_hbm, c_v, wsem.at[1])
        start(x_hbm, x_v, wsem.at[0])
        issue(wma_p)
        start(b1_hbm, b1_v, wsem.at[2])
        ctr[0] += 1
        issue(wq_p[:120])

        def layernorm(v):
            m = jnp.mean(v, axis=-1, keepdims=True)
            d = v - m
            var = jnp.mean(d * d, axis=-1, keepdims=True)
            return d / jnp.sqrt(var + EPS)

        wait(c_v, wsem.at[1])
        wait(x_v, wsem.at[0])
        wait(wma_v, wsem.at[3])
        cf = c_v[...].astype(jnp.float32)
        sc = jnp.broadcast_to(cf * jax.nn.sigmoid(cf), (8, D)).astype(jnp.bfloat16)
        x = jnp.broadcast_to(x_v[0].astype(jnp.float32), (8, D))
        moda = jnp.dot(sc, wma_v[...], preferred_element_type=jnp.float32)
        h = (layernorm(x) * (1.0 + moda[:, D:]) + moda[:, :D]).astype(jnp.bfloat16)

        issue(wq_p[120:])
        issue(wo_p[:96])
        wait(wq_v, wsem.at[5])
        row = lax.broadcasted_iota(jnp.int32, (GH, GR), 0)
        col = lax.broadcasted_iota(jnp.int32, (GH, GR), 1)
        mask = (col >= row * DH) & (col < (row + 1) * DH)
        for g in range(NG):
            if compute:
                q = jnp.dot(h, wq_v[:, g * GR:(g + 1) * GR], preferred_element_type=jnp.float32)
                qbd = jnp.where(mask, q, 0.0).astype(jnp.bfloat16)
                for u in range(UPG):
                    qbd_s[g * UPG + u] = qbd[:, u * UR:(u + 1) * UR]
            issue(wo_p[96 + g * 24:96 + (g + 1) * 24])
        ctr[0] = 0
        for t in range(L):
            issue_unit(kt_hbm, t, t % R)
        acc_s[...] = jnp.zeros(acc_s.shape, acc_s.dtype)
        wait(wo_v, wsem.at[6])

        def k_step(g, u, slot):
            wait(ring.at[slot], rsem.at[slot])
            if compute:
                s_s[...] += jnp.dot(qbd_s[g * UPG + u], ring[slot], preferred_element_type=jnp.float32)

        def softmax():
            s = s_s[...] * (DH ** -0.5)
            e = jnp.exp(s - jnp.max(s, axis=-1, keepdims=True))
            p_s[...] = (e / jnp.sum(e, axis=-1, keepdims=True)).astype(jnp.bfloat16)

        def v_step(g, u, slot):
            wait(ring.at[slot], rsem.at[slot])
            if compute:
                o = lax.dot_general(p_s[...], ring[slot], (((1,), (1,)), ((), ())),
                                    preferred_element_type=jnp.float32)
                r_ = lax.broadcasted_iota(jnp.int32, (GH, UR), 0) * DH
                c_ = lax.broadcasted_iota(jnp.int32, (GH, UR), 1) + u * UR
                o = jnp.where((c_ >= r_) & (c_ < r_ + DH), o, 0.0).astype(jnp.bfloat16)
                r0 = pl.multiple_of((g * UPG + u) * UR, UR)
                acc_s[...] += jnp.dot(o, wo_v[pl.ds(r0, UR), :], preferred_element_type=jnp.float32)

        def group(g, last):
            t0 = g * (2 * UPG)
            s_s[...] = jnp.zeros(s_s.shape, s_s.dtype)

            def a(u, _):
                issue_unit(kt_hbm, g * UPG + u + L, lax.rem(t0 + u + L, R))
                k_step(g, u, lax.rem(t0 + u, R))
            lax.fori_loop(0, UPG - L, a, None)

            def b(u, _):
                issue_unit(vt_hbm, g * UPG + u + L - UPG, lax.rem(t0 + u + L, R))
                k_step(g, u, lax.rem(t0 + u, R))
            lax.fori_loop(UPG - L, UPG, b, None)
            softmax()

            def c(u, _):
                issue_unit(vt_hbm, g * UPG + u + L, lax.rem(t0 + UPG + u + L, R))
                v_step(g, u, lax.rem(t0 + UPG + u, R))
            lax.fori_loop(0, UPG - L, c, None)
            if not last:
                def d(u, _):
                    issue_unit(kt_hbm, (g + 1) * UPG + u + L - UPG, lax.rem(t0 + UPG + u + L, R))
                    v_step(g, u, lax.rem(t0 + UPG + u, R))
                lax.fori_loop(UPG - L, UPG, d, None)

        lax.fori_loop(0, NG - 1, lambda g, _: group(g, False), None)
        group(NG - 1, True)

        ctr[0] = 0
        tail = wmb_p + w1_p + w2_p
        n_per = 32
        pos = 0
        for u in range(UPG - L, UPG):
            issue(tail[pos:pos + n_per])
            pos += n_per
            v_step(NG - 1, u, ((NG - 1) * 2 * UPG + UPG + u) % R)
        issue(tail[pos:])
        wait(wmb_v, wsem.at[4])
        modb = jnp.dot(sc, wmb_v[...], preferred_element_type=jnp.float32)
        ga, sb, cb, gb = (modb[:, i * D:(i + 1) * D] for i in range(4))
        attn = jnp.broadcast_to(jnp.sum(acc_s[...], axis=0, keepdims=True), (8, D))
        x1 = x + ga * attn
        h2 = (layernorm(x1) * (1.0 + cb) + sb).astype(jnp.bfloat16)
        wait(b1_v, wsem.at[2])
        if b1_mode == "2d":
            b1f = b1_v[...].astype(jnp.float32)
            b1 = jnp.concatenate([b1f[j:j + 1, :] for j in range(F // 128)], axis=1)
        else:
            b1 = b1_v[...].astype(jnp.float32).reshape(1, F)
        wait(w1_v, wsem.at[7])
        z = jnp.dot(h2, w1_v[...], preferred_element_type=jnp.float32) + b1
        sp = jnp.log1p(jnp.exp(-jnp.abs(z))) + jnp.where(z > 0, z, 0.0)
        act = (z * jnp.tanh(sp)).astype(jnp.bfloat16)
        wait(w2_v, wsem.at[8])
        y = jnp.dot(act, w2_v[...], preferred_element_type=jnp.float32)
        out = x1 + gb * y
        o_ref[0] = out[0:1, :].astype(o_ref.dtype)

    def fn(A_x, A_k_cache, A_v_cache, A_wq, A_wo, B_x, B_w1, B_b1, B_w2, c, w_mod):
        sk = A_k_cache.shape[2]
        w = min(4096, max(256, sk // 4))
        kt = jnp.swapaxes(A_k_cache, 2, 3).reshape(HD, sk)
        vt = jnp.swapaxes(A_v_cache, 2, 3).reshape(HD, sk)
        b1 = B_b1.reshape(F // 128, 128) if b1_mode == "2d" else B_b1
        bf = jnp.bfloat16
        hbm = pl.BlockSpec(memory_space=pltpu.HBM)
        kw = dict(disable_bounds_checks=True, disable_semaphore_checks=True, skip_device_barrier=True) if nochecks else {}
        return pl.pallas_call(
            kernel,
            out_shape=jax.ShapeDtypeStruct(A_x.shape, A_x.dtype),
            in_specs=[hbm] * 10,
            out_specs=pl.BlockSpec(memory_space=pltpu.VMEM),
            scratch_shapes=[
                pltpu.VMEM(A_x.shape, bf), pltpu.VMEM(c.shape, bf), pltpu.VMEM(b1.shape, bf),
                pltpu.VMEM((D, 2 * D), bf), pltpu.VMEM((D, 4 * D), bf), pltpu.VMEM((D, HD), bf),
                pltpu.VMEM((HD, D), bf), pltpu.VMEM((D, F), bf), pltpu.VMEM((F, D), bf),
                pltpu.VMEM((R, UR, w), bf), pltpu.VMEM((8, 6 * D), jnp.float32),
                pltpu.VMEM((NG * UPG, GH, UR), bf), pltpu.VMEM((GH, w), jnp.float32),
                pltpu.VMEM((GH, w), bf), pltpu.VMEM((8, D), jnp.float32),
                pltpu.SemaphoreType.DMA((9,)), pltpu.SemaphoreType.DMA((R,)),
            ],
            compiler_params=pltpu.CompilerParams(vmem_limit_bytes=100 * 1024 * 1024, **kw),
        )(A_x, kt, vt, A_wq, A_wo, B_w1, b1, B_w2, c, w_mod)

    return fn


_impl = make(kv_order="col")


@jax.jit
def pallas_adaLN_cond__sliding_block_cached__dense_activation_mish__decode_kernel(
    A_x, A_k_cache, A_v_cache, A_wq, A_wo, B_x, B_w1, B_b1, B_w2, c, w_mod):
    return _impl(A_x, A_k_cache, A_v_cache, A_wq, A_wo, B_x, B_w1, B_b1, B_w2, c, w_mod)
```

```python
import contextlib
import math

import jax
import jax.numpy as jnp
from jax import lax
from jax.experimental import pallas as pl
from jax.experimental.pallas import tpu as pltpu

D = 640
HQ = 32
DH = 192
F = 1536
HD = HQ * DH
GH = 8
GR = GH * DH
NG = HQ // GH
EPS = 1e-5


def make(UR=128, L=3, R=8, ks=(16, 16), vs=(24, 8), compute=True, tail_compute=True, nochecks=True,
         wq="cls", wm=((15, 15), 17), gb_tail=False, gb=(32, 7), wo_rows=32, w1=(16, 8), w2=(32, 13),
         w2_chunks=(768, 512, 256), tail=None, scopes=False, wo_mode="head", wo_step=13, wo_sub=2,
         w1_chunks=(1536,), wq_first=False):
    UPG = GR // UR
    scope = jax.named_scope if scopes else (lambda n: contextlib.nullcontext())
    n_head = 5 if gb_tail else 6
    AB = (0, 1)
    if tail is None:
        n1 = D // w1[0]
        seq = [("w1", 0, n1, AB)] + ([("gb", 0, D // gb[0], AB)] if gb_tail else [])
        seq += [("w2_%d" % i, 0, n // w2[0], AB) for i, n in enumerate(w2_chunks)]
        tail = [[("w1", 0, 28, AB)], [("w1", 28, n1, AB)] + seq[1:2]] + [[] for _ in range(L - 2)] + [seq[2:]]
    assert len(tail) == L + 1

    def kernel(x_hbm, kt_hbm, vt_hbm, wq_hbm, wo_hbm, w1_hbm, b1_hbm, w2_hbm, c_hbm, wm_hbm, o_ref,
               x_v, c_v, b1_v, wma_v, wmb_v, wq_v, wo_v, w1_v, w2_v, ring, qbd_s, s_s, p_s, acc_s,
               wsem, rsem, osem):
        sk = kt_hbm.shape[1]
        w = ring.shape[2]
        c0 = sk - w

        def start(src, dst, sem, q):
            pltpu.make_async_copy(src, dst, sem).start(priority=q)

        def wait(dst, sem):
            pltpu.make_async_copy(dst, dst, sem).wait()

        def issue_loop(fn, lo, hi, queues=AB):
            k = len(queues)
            assert (hi - lo) % k == 0, (lo, hi, queues)

            def body(i, _):
                for e, q in enumerate(queues):
                    fn(lo + i * k + e, q)
            if hi > lo:
                lax.fori_loop(0, (hi - lo) // k, body, None)

        def rows_fn(src, dst, sem, rows, step, row0=0, nrows=None, scol=0, dcol=0, ncol=None):
            nrows = dst.shape[0] if nrows is None else nrows
            ncol = dst.shape[1] if ncol is None else ncol
            n = nrows // rows
            per = n // math.gcd(n, step)

            def fn(j, q):
                blk = lax.rem(j * step + lax.div(j, per), n)
                r = pl.multiple_of(row0 + blk * rows, 8)
                start(src.at[pl.ds(r, rows), pl.ds(scol, ncol)], dst.at[pl.ds(r, rows), pl.ds(dcol, ncol)], sem, q)
            return fn

        def issue_unit(src, unit, slot, split, with_wo):
            base = pl.multiple_of(unit * UR, UR)
            offs = [sum(split[:i]) for i in range(len(split))]
            if not with_wo:
                for c in range(len(split)):
                    for r in range(UR // 8):
                        start(src.at[pl.ds(base + 8 * r, 8), pl.ds(c0 + offs[c] * 128, split[c] * 128)],
                              ring.at[slot, pl.ds(8 * r, 8), pl.ds(offs[c] * 128, split[c] * 128)], rsem.at[slot],
                              r % 2)
                return
            n_wo = UR // wo_rows
            per_c = n_wo // len(split)
            for c in range(len(split)):
                def body(i, _):
                    k = 0
                    for e in range(UR // 8 // wo_sub):
                        r = pl.multiple_of(i * (UR // wo_sub) + 8 * e, 8)
                        start(src.at[pl.ds(base + r, 8), pl.ds(c0 + offs[c] * 128, split[c] * 128)],
                              ring.at[slot, pl.ds(r, 8), pl.ds(offs[c] * 128, split[c] * 128)], rsem.at[slot], k % 2)
                        k += 1
                    for e in range(per_c // wo_sub):
                        r = pl.multiple_of(base + (c * per_c + i * (per_c // wo_sub) + e) * wo_rows, 8)
                        start(wo_hbm.at[pl.ds(r, wo_rows), :], wo_v.at[pl.ds(r, wo_rows), :], osem.at[unit],
                              (k + c) % 2)
                        k += 1
                lax.fori_loop(0, wo_sub, body, None)

        def layernorm(v):
            m = jnp.mean(v, axis=-1, keepdims=True)
            d = v - m
            var = jnp.mean(d * d, axis=-1, keepdims=True)
            return d / jnp.sqrt(var + EPS)

        def wq_fn(j, q):
            if wq == "cls":
                n = 2 * lax.div(j, 30) + lax.rem(j, 2) + 16 * lax.rem(lax.div(j, 2), 15)
                r, c = lax.div(n, 3), lax.rem(n, 3)
            elif wq == "cls1":
                n = lax.div(j, 15) + 16 * lax.rem(j, 15)
                r, c = lax.div(n, 3), lax.rem(n, 3)
            else:
                c = lax.div(j, 80)
                jj = lax.rem(j, 80)
                r = lax.rem(jj * wq + lax.div(jj, 80 // math.gcd(80, wq)), 80)
            r = pl.multiple_of(r * 8, 8)
            c = pl.multiple_of(c * 2048, 2048)
            start(wq_hbm.at[pl.ds(r, 8), pl.ds(c, 2048)], wq_v.at[pl.ds(r, 8), pl.ds(c, 2048)], wsem.at[5], q)

        parts = {}
        f0 = 0
        for i, n in enumerate(w1_chunks):
            parts["w1" + ("" if len(w1_chunks) == 1 else "_%d" % i)] = rows_fn(
                w1_hbm, w1_v, wsem.at[8 + len(w2_chunks) + i], w1[0], w1[1], scol=f0, dcol=f0, ncol=n)
            f0 += n
        r0 = 0
        for i, n in enumerate(w2_chunks):
            parts["w2_%d" % i] = rows_fn(w2_hbm, w2_v, wsem.at[8 + i], w2[0], w2[1], row0=r0, nrows=n)
            r0 += n
        assert r0 == F and f0 == F
        if gb_tail:
            parts["gb"] = rows_fn(wm_hbm, wmb_v, wsem.at[4], gb[0], gb[1], scol=5 * D)

        off = 0
        for i, n in enumerate(wm[0]):
            issue_loop(rows_fn(wm_hbm, wma_v, wsem.at[3], 8, wm[1], scol=off * 128, dcol=off * 128, ncol=n * 128),
                       0, D // 8)
            if i == 0:
                start(c_hbm, c_v, wsem.at[1], 0)
                start(x_hbm, x_v, wsem.at[0], 0)
                start(b1_hbm, b1_v, wsem.at[2], 0)
            off += n
        assert off == 5 * n_head
        issue_loop(wq_fn, 0, 120)

        with scope("h_wait"):
            wait(c_v, wsem.at[1])
            wait(x_v, wsem.at[0])
            wait(b1_v, wsem.at[2])
            wait(wma_v, wsem.at[3])
        with scope("h_mod"):
            cf = c_v[...].astype(jnp.float32)
            sc = jnp.broadcast_to(cf * jax.nn.sigmoid(cf), (8, D)).astype(jnp.bfloat16)
            x = jnp.broadcast_to(x_v[0].astype(jnp.float32), (8, D))
            mod = jnp.dot(sc, wma_v[...], preferred_element_type=jnp.float32)
            sa, ca, ga, sb, cb = (mod[:, i * D:(i + 1) * D] for i in range(5))
            h = (layernorm(x) * (1.0 + ca) + sa).astype(jnp.bfloat16)

        issue_loop(wq_fn, 120, 240)
        if wo_mode == "head":
            issue_loop(rows_fn(wo_hbm, wo_v, wsem.at[6], wo_rows, wo_step), 0, HD // wo_rows)
        lax.fori_loop(0, L, lambda t, _: issue_unit(kt_hbm, t, t, ks, wo_mode == "k"), None)
        if wo_mode == "head":
            wait(wo_v, wsem.at[6])
        acc_s[...] = jnp.zeros(acc_s.shape, acc_s.dtype)
        with scope("h_wait_wq"):
            wait(wq_v, wsem.at[5])

        def make_q(g):
            if compute:
                c_ = pl.multiple_of(g * GR, 128)
                q = jnp.dot(h, wq_v[:, pl.ds(c_, GR)], preferred_element_type=jnp.float32)
                row = lax.broadcasted_iota(jnp.int32, (GH, GR), 0) * DH
                col = lax.broadcasted_iota(jnp.int32, (GH, GR), 1)
                qbd_s[...] = jnp.where((col >= row) & (col < row + DH), q, 0.0).astype(jnp.bfloat16)

        def k_step(u, slot):
            wait(ring.at[slot], rsem.at[slot])
            if compute:
                r0 = pl.multiple_of(u * UR, UR)
                s_s[...] += jnp.dot(qbd_s[:, pl.ds(r0, UR)], ring[slot], preferred_element_type=jnp.float32)

        def softmax():
            s = s_s[...] * (DH ** -0.5)
            e = jnp.exp(s - jnp.max(s, axis=-1, keepdims=True))
            p_s[...] = (e / jnp.sum(e, axis=-1, keepdims=True)).astype(jnp.bfloat16)

        def v_step(g, u, slot):
            wait(ring.at[slot], rsem.at[slot])
            wo_u = wo_v.at[pl.ds(pl.multiple_of((g * UPG + u) * UR, UR), UR), :]
            if wo_mode != "head":
                wait(wo_u, osem.at[g * UPG + u])
            if compute:
                o = lax.dot_general(p_s[...], ring[slot], (((1,), (1,)), ((), ())),
                                    preferred_element_type=jnp.float32)
                r_ = lax.broadcasted_iota(jnp.int32, (GH, UR), 0) * DH
                c_ = lax.broadcasted_iota(jnp.int32, (GH, UR), 1) + u * UR
                o = jnp.where((c_ >= r_) & (c_ < r_ + DH), o, 0.0).astype(jnp.bfloat16)
                acc_s[...] += jnp.dot(o, wo_u[...], preferred_element_type=jnp.float32)

        def group(g, last):
            t0 = g * (2 * UPG)
            make_q(g)
            s_s[...] = jnp.zeros(s_s.shape, s_s.dtype)

            def a(u, _):
                issue_unit(kt_hbm, g * UPG + u + L, lax.rem(t0 + u + L, R), ks, wo_mode == "k")
                k_step(u, lax.rem(t0 + u, R))
            lax.fori_loop(0, UPG - L, a, None)

            def b(u, _):
                issue_unit(vt_hbm, g * UPG + u + L - UPG, lax.rem(t0 + u + L, R), vs, wo_mode == "v")
                k_step(u, lax.rem(t0 + u, R))
            lax.fori_loop(UPG - L, UPG, b, None)
            softmax()

            def c(u, _):
                issue_unit(vt_hbm, g * UPG + u + L, lax.rem(t0 + UPG + u + L, R), vs, wo_mode == "v")
                v_step(g, u, lax.rem(t0 + UPG + u, R))
            lax.fori_loop(0, UPG - L, c, None)
            if not last:
                def d(u, _):
                    issue_unit(kt_hbm, (g + 1) * UPG + u + L - UPG, lax.rem(t0 + UPG + u + L, R), ks, wo_mode == "k")
                    v_step(g, u, lax.rem(t0 + UPG + u, R))
                lax.fori_loop(UPG - L, UPG, d, None)

        with scope("main"):
            lax.fori_loop(0, NG - 1, lambda g, _: group(g, False), None)
            group(NG - 1, True)

        def issue_tail(i):
            for name, lo, hi, queues in tail[i]:
                issue_loop(parts[name], lo, hi, queues)

        def last_steps(i, _):
            for k in range(L):
                if tail[k]:
                    pl.when(i == k)(lambda k=k: issue_tail(k))
            u = UPG - L + i
            v_step(NG - 1, u, lax.rem((NG - 1) * 2 * UPG + UPG + u, R))
        with scope("t_vsteps"):
            lax.fori_loop(0, L, last_steps, None)
        with scope("t_issue_rest"):
            issue_tail(L)
        if not tail_compute:
            f0 = 0
            for i, n in enumerate(w1_chunks):
                wait(w1_v.at[:, pl.ds(f0, n)], wsem.at[8 + len(w2_chunks) + i])
                f0 += n
            if gb_tail:
                wait(wmb_v, wsem.at[4])
            r0 = 0
            for i, n in enumerate(w2_chunks):
                wait(w2_v.at[pl.ds(r0, n), :], wsem.at[8 + i])
                r0 += n
            o_ref[0] = x[0:1].astype(o_ref.dtype)
            return
        with scope("t_ln"):
            attn = jnp.broadcast_to(jnp.sum(acc_s[...], axis=0, keepdims=True), (8, D))
            x1 = x + ga * attn
            h2 = (layernorm(x1) * (1.0 + cb) + sb).astype(jnp.bfloat16)
            b1f = b1_v[...].astype(jnp.float32)
            b1 = jnp.concatenate([b1f[j:j + 1, :] for j in range(F // 128)], axis=1)
        acts = []
        f0 = 0
        for i, n in enumerate(w1_chunks):
            with scope("t_wait_w1_%d" % i):
                wait(w1_v.at[:, pl.ds(f0, n)], wsem.at[8 + len(w2_chunks) + i])
            with scope("t_w1_%d" % i):
                z = jnp.dot(h2, w1_v[:, f0:f0 + n], preferred_element_type=jnp.float32) + b1[:, f0:f0 + n]
                sp = jnp.log1p(jnp.exp(-jnp.abs(z))) + jnp.where(z > 0, z, 0.0)
                acts.append((z * jnp.tanh(sp)).astype(jnp.bfloat16))
            f0 += n
        act = jnp.concatenate(acts, axis=1)

        def gate_b():
            if not gb_tail:
                return mod[:, 5 * D:]
            with scope("t_wait_gb"):
                wait(wmb_v, wsem.at[4])
            with scope("t_gb"):
                return jnp.dot(sc, wmb_v[...], preferred_element_type=jnp.float32)

        gb_last = tail[-1][-1][0] == "gb"
        if not gb_last:
            gbv = gate_b()
        assert not gb_last
        qbd_s[:, 0:F] = act
        acc_s[...] = jnp.zeros(acc_s.shape, acc_s.dtype)
        starts = [sum(w2_chunks[:i]) for i in range(len(w2_chunks))]

        def w2_part(i):
            r0, n = starts[i], w2_chunks[i]
            with scope("t_wait_w2_%d" % i):
                wait(w2_v.at[pl.ds(r0, n), :], wsem.at[8 + i])
            with scope("t_w2_%d" % i):
                return acc_s[...] + jnp.dot(qbd_s[:, r0:r0 + n], w2_v[r0:r0 + n, :],
                                            preferred_element_type=jnp.float32)

        def w2_steps(i, _):
            for k in range(len(w2_chunks) - 1):
                @pl.when(i == k)
                def _(k=k):
                    acc_s[...] = w2_part(k)
        if len(w2_chunks) > 1:
            lax.fori_loop(0, len(w2_chunks) - 1, w2_steps, None)
        y = w2_part(len(w2_chunks) - 1)
        o_ref[0] = (x1 + gbv * y)[0:1, :].astype(o_ref.dtype)

    def fn(A_x, A_k_cache, A_v_cache, A_wq, A_wo, B_x, B_w1, B_b1, B_w2, c, w_mod):
        sk = A_k_cache.shape[2]
        w = min(4096, max(256, sk // 4))
        kt = jnp.swapaxes(A_k_cache, 2, 3).reshape(HD, sk)
        vt = jnp.swapaxes(A_v_cache, 2, 3).reshape(HD, sk)
        b1 = B_b1.reshape(F // 128, 128)
        bf = jnp.bfloat16
        hbm = pl.BlockSpec(memory_space=pltpu.HBM)
        kw = dict(disable_bounds_checks=True, disable_semaphore_checks=True, skip_device_barrier=True) if nochecks else {}
        return pl.pallas_call(
            kernel,
            out_shape=jax.ShapeDtypeStruct(A_x.shape, A_x.dtype),
            in_specs=[hbm] * 10,
            out_specs=pl.BlockSpec(memory_space=pltpu.VMEM),
            scratch_shapes=[
                pltpu.VMEM(A_x.shape, bf), pltpu.VMEM(c.shape, bf), pltpu.VMEM(b1.shape, bf),
                pltpu.VMEM((D, n_head * D), bf), pltpu.VMEM((D, D), bf), pltpu.VMEM((D, HD), bf),
                pltpu.VMEM((HD, D), bf), pltpu.VMEM((D, F), bf), pltpu.VMEM((F, D), bf),
                pltpu.VMEM((R, UR, w), bf),
                pltpu.VMEM((GH, GR), bf), pltpu.VMEM((GH, w), jnp.float32),
                pltpu.VMEM((GH, w), bf), pltpu.VMEM((8, D), jnp.float32),
                pltpu.SemaphoreType.DMA((8 + len(w2_chunks) + len(w1_chunks),)), pltpu.SemaphoreType.DMA((R,)),
                pltpu.SemaphoreType.DMA((NG * UPG,)),
            ],
            compiler_params=pltpu.CompilerParams(vmem_limit_bytes=100 * 1024 * 1024, **kw),
        )(A_x, kt, vt, A_wq, A_wo, B_w1, b1, B_w2, c, w_mod)

    return fn


_impl = make(UR=256, L=2)


@jax.jit
def pallas_adaLN_cond__sliding_block_cached__dense_activation_mish__decode_kernel(
    A_x, A_k_cache, A_v_cache, A_wq, A_wo, B_x, B_w1, B_b1, B_w2, c, w_mod):
    return _impl(A_x, A_k_cache, A_v_cache, A_wq, A_wo, B_x, B_w1, B_b1, B_w2, c, w_mod)
```

```python
import math

import jax
import jax.numpy as jnp
from jax import lax
from jax.experimental import pallas as pl
from jax.experimental.pallas import tpu as pltpu

D = 640
HQ = 32
DH = 192
F = 1536
HD = HQ * DH
EPS = 1e-5

GH = 8
GR = GH * DH
NG = HQ // GH
UR = 256
UPG = GR // UR
AHEAD = 2
SLOTS = 4

TILE = 128
K_SPLIT = (16, 16)
V_SPLIT = (24, 8)
MOD_SPLIT = (15, 15)
W2_CHUNKS = ((1152, 18, (0, 1)), (256, 3, (1,)), (128, 1, (1,)))
BOTH = (0, 1)

SEM_X, SEM_C, SEM_B1, SEM_MOD, SEM_WQ, SEM_WO, SEM_W1, SEM_W2 = range(8)


def _layernorm(v):
    d = v - jnp.mean(v, axis=-1, keepdims=True)
    return d / jnp.sqrt(jnp.mean(d * d, axis=-1, keepdims=True) + EPS)


def _head_mask(shape, col0):
    lo = lax.broadcasted_iota(jnp.int32, shape, 0) * DH
    col = lax.broadcasted_iota(jnp.int32, shape, 1) + col0
    return (col >= lo) & (col < lo + DH)


def _dot(a, b):
    return jnp.dot(a, b, preferred_element_type=jnp.float32)


def _kernel(x_hbm, kt_hbm, vt_hbm, wq_hbm, wo_hbm, w1_hbm, b1_hbm, w2_hbm, c_hbm, wm_hbm, o_ref,
            x_v, c_v, b1_v, wm_v, wq_v, wo_v, w1_v, w2_v, ring,
            q_s, s_s, p_s, act_s, acc_s, wsem, rsem):
    win0 = kt_hbm.shape[1] - ring.shape[2]

    def start(src, dst, sem, priority):
        pltpu.make_async_copy(src, dst, sem).start(priority=priority)

    def wait(dst, sem):
        pltpu.make_async_copy(dst, dst, sem).wait()

    def issue(copy, lo, hi, priorities=BOTH):
        k = len(priorities)
        assert (hi - lo) % k == 0

        def body(i, _):
            for e, priority in enumerate(priorities):
                copy(lo + i * k + e, priority)

        lax.fori_loop(0, (hi - lo) // k, body, None)

    def row_blocks(src, dst, sem, rows, step, drift=1, row0=0, nrows=None, col0=0, ncols=None):
        nrows = dst.shape[0] if nrows is None else nrows
        ncols = dst.shape[1] if ncols is None else ncols
        n = nrows // rows
        cycle = n // math.gcd(n, step)
        assert sorted((j * step + drift * (j // cycle)) % n for j in range(n)) == list(range(n))

        def copy(j, priority):
            blk = lax.rem(j * step + drift * lax.div(j, cycle), n)
            idx = (pl.ds(pl.multiple_of(row0 + blk * rows, 8), rows), pl.ds(col0, ncols))
            start(src.at[idx], dst.at[idx], sem, priority)

        return copy, 0, n

    def wq_copy(j, priority):
        n = 2 * lax.div(j, 30) + lax.rem(j, 2) + 16 * lax.rem(lax.div(j, 2), 15)
        idx = (pl.ds(pl.multiple_of(lax.div(n, 3) * 8, 8), 8),
               pl.ds(pl.multiple_of(lax.rem(n, 3) * 2048, 2048), 2048))
        start(wq_hbm.at[idx], wq_v.at[idx], wsem.at[SEM_WQ], priority)

    def issue_unit(src, split, unit, slot):
        row0 = pl.multiple_of(unit * UR, UR)
        col = 0
        for tiles in split:
            n = tiles * TILE
            for r in range(UR // 8):
                start(src.at[pl.ds(row0 + 8 * r, 8), pl.ds(win0 + col, n)],
                      ring.at[slot, pl.ds(8 * r, 8), pl.ds(col, n)], rsem.at[slot], r % 2)
            col += n

    col = 0
    for i, tiles in enumerate(MOD_SPLIT):
        issue(*row_blocks(wm_hbm, wm_v, wsem.at[SEM_MOD], 8, 17, col0=col, ncols=tiles * TILE))
        col += tiles * TILE
        if i == 0:
            start(c_hbm, c_v, wsem.at[SEM_C], 0)
            start(x_hbm, x_v, wsem.at[SEM_X], 0)
            start(b1_hbm, b1_v, wsem.at[SEM_B1], 0)
    issue(wq_copy, 0, 120)

    wait(c_v, wsem.at[SEM_C])
    wait(x_v, wsem.at[SEM_X])
    wait(b1_v, wsem.at[SEM_B1])
    wait(wm_v, wsem.at[SEM_MOD])
    c = c_v[...].astype(jnp.float32)
    silu_c = jnp.broadcast_to(c * jax.nn.sigmoid(c), (GH, D)).astype(jnp.bfloat16)
    x = jnp.broadcast_to(x_v[0].astype(jnp.float32), (GH, D))
    mod = _dot(silu_c, wm_v[...])
    sa, ca, ga, sb, cb, gb = (mod[:, i * D:(i + 1) * D] for i in range(6))
    h = (_layernorm(x) * (1.0 + ca) + sa).astype(jnp.bfloat16)

    issue(wq_copy, 120, 240)
    issue(*row_blocks(wo_hbm, wo_v, wsem.at[SEM_WO], 32, 64, drift=13))
    lax.fori_loop(0, AHEAD, lambda t, _: issue_unit(kt_hbm, K_SPLIT, t, t), None)
    acc_s[...] = jnp.zeros(acc_s.shape, acc_s.dtype)
    wait(wq_v, wsem.at[SEM_WQ])
    wait(wo_v, wsem.at[SEM_WO])

    w1_copy, _, w1_n = row_blocks(w1_hbm, w1_v, wsem.at[SEM_W1], 16, 8)
    w2_rows = [sum(n for n, _, _ in W2_CHUNKS[:i]) for i in range(len(W2_CHUNKS))]
    w2_issue = [
        row_blocks(w2_hbm, w2_v, wsem.at[SEM_W2 + i], 32, step, row0=w2_rows[i], nrows=n) + (priorities,)
        for i, (n, step, priorities) in enumerate(W2_CHUNKS)
    ]
    mlp_issue = ([(w1_copy, 0, 28)], [(w1_copy, 28, w1_n), w2_issue[0]])
    assert len(mlp_issue) == AHEAD

    def group(g, _):
        def slot(u):
            return lax.rem(g * (2 * UPG) + u, SLOTS)

        def k_step(u):
            wait(ring.at[slot(u)], rsem.at[slot(u)])
            s_s[...] += _dot(q_s[:, pl.ds(pl.multiple_of(u * UR, UR), UR)], ring[slot(u)])

        def v_step(u):
            wait(ring.at[slot(UPG + u)], rsem.at[slot(UPG + u)])
            o = lax.dot_general(p_s[...], ring[slot(UPG + u)], (((1,), (1,)), ((), ())),
                                preferred_element_type=jnp.float32)
            o = jnp.where(_head_mask(o.shape, u * UR), o, 0.0).astype(jnp.bfloat16)
            acc_s[...] += _dot(o, wo_v[pl.ds(pl.multiple_of((g * UPG + u) * UR, UR), UR), :])

        q = _dot(h, wq_v[:, pl.ds(pl.multiple_of(g * GR, GR), GR)])
        q_s[...] = jnp.where(_head_mask(q.shape, 0), q, 0.0).astype(jnp.bfloat16)
        s_s[...] = jnp.zeros(s_s.shape, s_s.dtype)

        def k_then_k(u, _):
            issue_unit(kt_hbm, K_SPLIT, g * UPG + u + AHEAD, slot(u + AHEAD))
            k_step(u)

        def k_then_v(u, _):
            issue_unit(vt_hbm, V_SPLIT, g * UPG + u + AHEAD - UPG, slot(u + AHEAD))
            k_step(u)

        def v_then_v(u, _):
            issue_unit(vt_hbm, V_SPLIT, g * UPG + u + AHEAD, slot(UPG + u + AHEAD))
            v_step(u)

        def v_then_next(u, _):
            @pl.when(g < NG - 1)
            def _():
                issue_unit(kt_hbm, K_SPLIT, g * UPG + u + AHEAD, slot(UPG + u + AHEAD))

            for i, items in enumerate(mlp_issue):
                @pl.when((g == NG - 1) & (u == UPG - AHEAD + i))
                def _(items=items):
                    for item in items:
                        issue(*item)

            v_step(u)

        lax.fori_loop(0, UPG - AHEAD, k_then_k, None)
        lax.fori_loop(UPG - AHEAD, UPG, k_then_v, None)
        s = s_s[...] * (DH ** -0.5)
        e = jnp.exp(s - jnp.max(s, axis=-1, keepdims=True))
        p_s[...] = (e / jnp.sum(e, axis=-1, keepdims=True)).astype(jnp.bfloat16)
        lax.fori_loop(0, UPG - AHEAD, v_then_v, None)
        lax.fori_loop(UPG - AHEAD, UPG, v_then_next, None)

    lax.fori_loop(0, NG, group, None)
    for item in w2_issue[1:]:
        issue(*item)

    attn = jnp.broadcast_to(jnp.sum(acc_s[...], axis=0, keepdims=True), (GH, D))
    x1 = x + ga * attn
    h2 = (_layernorm(x1) * (1.0 + cb) + sb).astype(jnp.bfloat16)
    b1 = b1_v[...].astype(jnp.float32)
    b1 = jnp.concatenate([b1[j:j + 1, :] for j in range(F // TILE)], axis=1)
    wait(w1_v, wsem.at[SEM_W1])
    z = _dot(h2, w1_v[...]) + b1
    softplus = jnp.log1p(jnp.exp(-jnp.abs(z))) + jnp.where(z > 0, z, 0.0)
    act_s[...] = (z * jnp.tanh(softplus)).astype(jnp.bfloat16)
    acc_s[...] = jnp.zeros(acc_s.shape, acc_s.dtype)

    def add_w2_chunk(i):
        rows = pl.ds(w2_rows[i], W2_CHUNKS[i][0])
        wait(w2_v.at[rows, :], wsem.at[SEM_W2 + i])
        return acc_s[...] + _dot(act_s[:, rows], w2_v[rows, :])

    def w2_step(i, _):
        for k in range(len(W2_CHUNKS) - 1):
            @pl.when(i == k)
            def _(k=k):
                acc_s[...] = add_w2_chunk(k)

    lax.fori_loop(0, len(W2_CHUNKS) - 1, w2_step, None)
    y = add_w2_chunk(len(W2_CHUNKS) - 1)
    o_ref[0] = (x1 + gb * y)[0:1, :].astype(o_ref.dtype)


@jax.jit
def pallas_adaLN_cond__sliding_block_cached__dense_activation_mish__decode_kernel(
    A_x: jax.Array,
    A_k_cache: jax.Array,
    A_v_cache: jax.Array,
    A_wq: jax.Array,
    A_wo: jax.Array,
    B_x: jax.Array,
    B_w1: jax.Array,
    B_b1: jax.Array,
    B_w2: jax.Array,
    c: jax.Array,
    w_mod: jax.Array,
):
    del B_x
    sk = A_k_cache.shape[2]
    w = min(4096, max(256, sk // 4))
    assert A_x.shape == (1, 1, D) and A_k_cache.shape == A_v_cache.shape == (1, HQ, sk, DH)
    assert w == sum(K_SPLIT) * TILE == sum(V_SPLIT) * TILE and sk % TILE == 0
    kt = jnp.swapaxes(A_k_cache, 2, 3).reshape(HD, sk)
    vt = jnp.swapaxes(A_v_cache, 2, 3).reshape(HD, sk)
    b1 = B_b1.reshape(F // TILE, TILE)

    bf16, f32 = jnp.bfloat16, jnp.float32
    return pl.pallas_call(
        _kernel,
        out_shape=jax.ShapeDtypeStruct(A_x.shape, A_x.dtype),
        in_specs=[pl.BlockSpec(memory_space=pltpu.HBM)] * 10,
        out_specs=pl.BlockSpec(memory_space=pltpu.VMEM),
        scratch_shapes=[
            *(pltpu.VMEM(a.shape, a.dtype) for a in (A_x, c, b1, w_mod, A_wq, A_wo, B_w1, B_w2)),
            pltpu.VMEM((SLOTS, UR, w), kt.dtype),
            pltpu.VMEM((GH, GR), bf16),
            pltpu.VMEM((GH, w), f32),
            pltpu.VMEM((GH, w), bf16),
            pltpu.VMEM((GH, F), bf16),
            pltpu.VMEM((GH, D), f32),
            pltpu.SemaphoreType.DMA((SEM_W2 + len(W2_CHUNKS),)),
            pltpu.SemaphoreType.DMA((SLOTS,)),
        ],
        compiler_params=pltpu.CompilerParams(
            vmem_limit_bytes=64 * 1024 * 1024, disable_semaphore_checks=True),
    )(A_x, kt, vt, A_wq, A_wo, B_w1, b1, B_w2, c, w_mod)
```
